```python
import jax
import jax.numpy as jnp

def _softmax(x, axis=-1):
    return jax.nn.softmax(x, axis=axis)
def _gelu(x):
    return jax.nn.gelu(x, approximate=True)
def _silu(x):
    return jax.nn.silu(x)
def _sigmoid(x):
    return jax.nn.sigmoid(x)
def _layernorm(x, axis=-1, eps=1e-5):
    m = jnp.mean(x, axis=axis, keepdims=True)
    v = jnp.var(x, axis=axis, keepdims=True)
    return (x - m) / jnp.sqrt(v + eps)
def _scatter_add(tgt, idx, src, axis=0):
    return tgt.at[idx].add(src)
def _segment_sum(src, seg, n):
    return jax.ops.segment_sum(src, seg, n)
class _Rng:
    def __init__(self, key):
        self._k = key
    def _next(self):
        self._k, sub = jax.random.split(self._k)
        return sub
    def normal(self, shape):
        return jax.random.normal(self._next(), shape, dtype=jnp.bfloat16)
    def randint(self, lo, hi, shape):
        return jax.random.randint(self._next(), shape, lo, hi, dtype=jnp.int32)
    def uniform(self, shape, lo=0.0, hi=1.0):
        return jax.random.uniform(self._next(), shape, jnp.bfloat16, lo, hi)
    def permutation(self, n):
        return jax.random.permutation(self._next(), n)


kernel_name = 'parallel_sum__linear_kernel_hedgehog__glu_gated_bilinear__prompt'

def _fwd_setup_inputs():
    _rng = _Rng(jax.random.key(int.from_bytes(__import__("os").urandom(4), "little")))
    _w = (lambda a: (lambda t: t.astype(jnp.bfloat16) if jnp.issubdtype(t.dtype, jnp.floating) else t)(jnp.asarray(a)))
    def _A_setup():
        B, S, D, H = 1, 2048, 512, 32
        Dh = D // H
        return {
            "x": _w((lambda *s: _rng.normal(s) * 0.05)(B, S, D)),
            "wqkv": _w((lambda *s: _rng.normal(s) * 0.05)(D, 3 * D)),
            "w_phi": _w((lambda *s: _rng.normal(s) * 0.05)(H, Dh, Dh) * (Dh ** -0.5)),
            "wo": _w((lambda *s: _rng.normal(s) * 0.05)(D, D)),
        }
    _A_in = _A_setup()

    def _B_setup():
        B, S, D, F = 1, 2048, 512, 1792
        return {
            "x": _w((lambda *s: _rng.normal(s) * 0.05)(B, S, D)),
            "w_gate": _w((lambda *s: _rng.normal(s) * 0.05)(D, F) * (D ** -0.5)),
            "w_up": _w((lambda *s: _rng.normal(s) * 0.05)(D, F) * (D ** -0.5)),
            "w_down": _w((lambda *s: _rng.normal(s) * 0.05)(F, D) * (F ** -0.5)),
        }
    _B_in = _B_setup()

    return {
        "A_x": _A_in["x"],
        "A_wqkv": _A_in["wqkv"],
        "A_w_phi": _A_in["w_phi"],
        "A_wo": _A_in["wo"],
        "B_x": _B_in["x"],
        "B_w_gate": _B_in["w_gate"],
        "B_w_up": _B_in["w_up"],
        "B_w_down": _B_in["w_down"],
    }

def _fwd_reference(A_x, A_wqkv, A_w_phi, A_wo, B_x, B_w_gate, B_w_up, B_w_down):
    def _A_ref(x, wqkv, w_phi, wo):
        B, S, D = x.shape
        H = 32; Dh = D // H
        qkv = (lambda x, *d: x.transpose(*d))((x @ wqkv).reshape(B, S, 3, H, Dh), 2, 0, 3, 1, 4)
        q, k, v = qkv[0], qkv[1], qkv[2]
        pq = jnp.einsum("bhsd,hdf->bhsf", q, w_phi)
        pk = jnp.einsum("bhsd,hdf->bhsf", k, w_phi)
        phi_q = jnp.concatenate([_softmax(pq, axis=-1), _softmax(-pq, axis=-1)], axis=-1)
        phi_k = jnp.concatenate([_softmax(pk, axis=-1), _softmax(-pk, axis=-1)], axis=-1)
        kv = jnp.einsum("bhsf,bhsd->bhfd", phi_k, v)
        z  = jnp.einsum("bhsf->bhf", phi_k)
        num = jnp.einsum("bhqf,bhfd->bhqd", phi_q, kv)
        den = jnp.einsum("bhqf,bhf->bhq", phi_q, z)[..., None] + 1e-6
        o = num / den
        return (lambda x, *d: x.transpose(*d))(o, 0, 2, 1, 3).reshape(B, S, D) @ wo

    def _B_ref(x, w_gate, w_up, w_down):
        g = jnp.einsum("bsd,df->bsf", x, w_gate)
        u = jnp.einsum("bsd,df->bsf", x, w_up)
        h = g * u
        return jnp.einsum("bsf,fd->bsd", h, w_down)

    x = A_x
    xn = _layernorm(x, axis=-1)
    return x + _A_ref(xn, A_wqkv, A_w_phi, A_wo) + _B_ref(xn, B_w_gate, B_w_up, B_w_down)


def setup_inputs():
    _inp = _fwd_setup_inputs()
    _gk = jax.random.fold_in(jax.random.key(int.from_bytes(__import__("os").urandom(4), "little")), 2**31 - 1)
    _shapes = [[1, 2048, 512]]
    _dtypes = ['bfloat16']
    _gks = jax.random.split(_gk, len(_shapes))
    _gs = [jax.random.normal(k, s, dtype=jnp.dtype(d)) * 0.05 for k, s, d in zip(_gks, _shapes, _dtypes)]
    _inp["grad_out"] = _gs[0]
    return _inp

def reference(A_x, A_wqkv, A_w_phi, A_wo, B_w_gate, B_w_up, B_w_down, B_x, grad_out):
    _const = dict(B_x=B_x)
    def _f(*_d):
        return _fwd_reference(**{'A_x': _d[0], 'A_wqkv': _d[1], 'A_w_phi': _d[2], 'A_wo': _d[3], 'B_w_gate': _d[4], 'B_w_up': _d[5], 'B_w_down': _d[6], **_const})
    _out, _vjp = jax.vjp(_f, A_x, A_wqkv, A_w_phi, A_wo, B_w_gate, B_w_up, B_w_down)
    _grads = _vjp(grad_out)
    _out0 = jnp.asarray(_out)
    return (_out0, *[jnp.asarray(_g) for _g in _grads])
```

```python
import jax
import jax.numpy as jnp
from jax import lax
import jax.experimental.pallas as pl
import jax.experimental.pallas.tpu as pltpu

S, D, F, H, DH = 2048, 512, 1792, 32, 16
NG = 4
T = 256
NTL = S // T
NLT = T // 128
C0 = 512
NC0 = S // C0
EPS_LN = 1e-5
EPS_DEN = 1e-6
SCOPES = False

f32, bf16 = jnp.float32, jnp.bfloat16
NN = (((1,), (0,)), ((), ()))
NT = (((1,), (1,)), ((), ()))
TN = (((0,), (0,)), ((), ()))
TT = (((0,), (1,)), ((), ()))


def _dot(a, b, dn):
    return lax.dot_general(a, b, dn, preferred_element_type=f32)


def _iota(shape, dim):
    return lax.broadcasted_iota(jnp.int32, shape, dim)


def _onehot(cond):
    return jnp.where(cond, 1.0, 0.0).astype(bf16)


def _pm():
    r_i, c_i = _iota((128, 128), 0), _iota((128, 128), 1)
    return _onehot(c_i == (r_i % 8) * 16 + r_i // 8)


def _pmT():
    r_i, c_i = _iota((128, 128), 0), _iota((128, 128), 1)
    return _onehot(r_i == (c_i % 8) * 16 + c_i // 8)


def _mask_kv():
    return (_iota((256, 128), 0) % 8) == (_iota((256, 128), 1) % 8)


def _lh():
    return _onehot(_iota((D, H), 0) // DH == _iota((D, H), 1))


def _mask_d():
    return (_iota((D, 256), 0) % DH) == (_iota((D, 256), 1) // DH)


def _e2():
    return _onehot(_iota((256, 128), 0) % DH == _iota((256, 128), 1) // 8)


def _tile_lanes(a):
    return jnp.concatenate([a] * NLT, axis=1)


def _interleave(mxu_tasks, vpu_tasks):
    nm, nv = len(mxu_tasks), len(vpu_tasks)
    done = 0
    for k, task in enumerate(mxu_tasks):
        task()
        if k < nm - 1:
            upto = min((nv * (k + 1) + nm - 2) // (nm - 1), nv)
            while done < upto:
                vpu_tasks[done]()
                done += 1
    assert done == nv


def _loop(name, n, body):
    if SCOPES:
        with jax.named_scope(name):
            lax.fori_loop(0, n, body, 0)
    else:
        lax.fori_loop(0, n, body, 0)


def _kernel(x_hbm, wqkv_hbm, wphi_hbm, wo_hbm, wg_hbm, wu_hbm, wd_hbm, dout_hbm,
            out_hbm, gx_hbm, dwqkv_hbm, dwphi_hbm, dwo_hbm, dwg_hbm, dwu_hbm, dwd_hbm,
            x_v, wqkv_v, wphi_v, wo_v, wg_v, wu_v, wd_v, dout_v,
            wpT_v, wop_v, phi_v,
            xn_v, xnT_v, mean_v, rstd_v,
            bufa_v, bufb_v, mm_v, phq_v, phk_v, vT_v,
            gu_v, h_v, part_v, dxb_v,
            z_acc, lhs_v, kvm_v, zcol_v,
            oT_v, dyT_v, dn_v, dd_v,
            dz_acc, dkvm_v, dkvmT_v,
            g_acc, dwo_acc, dwd_acc,
            out_v, gx_v, dwqkv_v, dwphi_v, dwo_v, dwg_v, dwu_v, dwd_v,
            pad_s, in_sems, x_sems, out_sems):
    def cp_x(c):
        rows = pl.ds(pl.multiple_of(c * C0, C0), C0)
        return pltpu.make_async_copy(x_hbm.at[0, rows], x_v.at[rows], x_sems.at[c])

    cp_wqkv = pltpu.make_async_copy(wqkv_hbm, wqkv_v, in_sems.at[0])
    cp_wphi = pltpu.make_async_copy(wphi_hbm, wphi_v, in_sems.at[1])
    cp_wg = pltpu.make_async_copy(wg_hbm, wg_v, in_sems.at[2])
    cp_wu = pltpu.make_async_copy(wu_hbm, wu_v, in_sems.at[3])
    cp_wd = pltpu.make_async_copy(wd_hbm, wd_v, in_sems.at[4])
    cp_wo = pltpu.make_async_copy(wo_hbm, wo_v, in_sems.at[5])
    cp_do = pltpu.make_async_copy(dout_hbm.at[0], dout_v, in_sems.at[6])
    cp_wphi.start()
    cp_wqkv.start()
    cp_x(0).start()

    pad_s[0] = NTL
    z_acc[...] = jnp.zeros(z_acc.shape, f32)
    dz_acc[...] = jnp.zeros(dz_acc.shape, f32)

    def fence(v, refs):
        pad = pad_s[0]
        for r in refs:
            if r.dtype == bf16:
                r[pad, 0:16, 0:128] = jnp.concatenate([v, v], axis=0).astype(bf16)
            else:
                r[pad, 0:8, 0:128] = v

    def ln_chunk(c):
        RC = 32
        for s in range(C0 // RC):
            rows = pl.ds(pl.multiple_of(c * C0 + s * RC, RC), RC)
            x = x_v[rows, :].astype(f32)
            m = jnp.mean(x, axis=1, keepdims=True)
            xc = x - m
            var = jnp.mean(xc * xc, axis=1, keepdims=True)
            rstd = lax.rsqrt(var + EPS_LN)
            mean_v[rows, :] = m
            rstd_v[rows, :] = rstd
            xn_v[rows, :] = (xc * rstd).astype(bf16)
        for s in range(C0 // T):
            rows = pl.ds(pl.multiple_of(c * C0 + s * T, T), T)
            xnT_v[c * (C0 // T) + s] = xn_v[rows, :].T

    cp_wphi.wait()
    cp_wqkv.wait()
    cp_x(0).wait()
    for c in range(1, NC0):
        cp_x(c).start()

    wt = wphi_v[...].reshape(256, H)
    bmat = jnp.where(_mask_d(), _dot(_lh(), wt, NT), 0.0).astype(bf16)
    mask_h = (_iota((D, 128), 1) % 8) == ((_iota((D, 128), 0) // DH) % 8)
    phi = jnp.where(mask_h, _dot(bmat, _e2(), NN), 0.0).astype(bf16)
    phi_v[...] = phi
    pm = _pm()
    for g in range(NG):
        ph_g = phi[g * 128:(g + 1) * 128, :]
        wq_g = wqkv_v[:, g * 128:(g + 1) * 128]
        wk_g = wqkv_v[:, D + g * 128:D + (g + 1) * 128]
        wv_g = wqkv_v[:, 2 * D + g * 128:2 * D + (g + 1) * 128]
        wpT_v[2 * D + g * 128:2 * D + (g + 1) * 128, :] = _dot(pm, wv_g, NT).astype(bf16)
        wpT_v[g * 128:(g + 1) * 128, :] = _dot(ph_g, wq_g, TT).astype(bf16)
        wpT_v[D + g * 128:D + (g + 1) * 128, :] = _dot(ph_g, wk_g, TT).astype(bf16)
    ln_chunk(0)
    cp_x(1).wait()
    cp_wg.start()
    cp_wu.start()
    cp_wd.start()
    cp_do.start()
    cp_wo.start()

    def loop0(c, carry):
        @pl.when(jnp.logical_and(c >= 1, c + 1 < NC0))
        def _():
            cp_x(c + 1).wait()

        rows = pl.ds(pl.multiple_of(c * C0, C0), C0)
        pT = _dot(wpT_v[...], xn_v[rows, :], NT)
        for s in range(C0 // T):
            t = c * (C0 // T) + s
            p = pT[0:2 * D, s * T:(s + 1) * T]
            bufa_v[t] = p
            p4 = p.reshape(2 * NG, DH, 8, T)
            mm_v[t, 0] = jnp.max(p4, axis=1)
            mm_v[t, 1] = jnp.min(p4, axis=1)
            vT_v[t] = pT[2 * D:3 * D, s * T:(s + 1) * T].astype(bf16)
        ln_chunk(jnp.minimum(c + 1, NC0 - 1))
        return carry

    _loop("L0", NC0, loop0)
    cp_wg.wait()
    cp_wu.wait()
    cp_wd.wait()
    cp_wo.wait()
    cp_do.wait()
    for g in range(NG):
        wop_v[g * 128:(g + 1) * 128, :] = _dot(_pm(), wo_v[g * 128:(g + 1) * 128, :], NN).astype(bf16)

    FBLK = ((0, 512), (512, 1024), (1024, 1536), (1536, 1792))

    def loop1(i, carry):
        rows = pl.ds(pl.multiple_of(i * T, T), T)

        def gu_task(a, b):
            def f():
                xn = xn_v[rows, :]
                gg = _dot(xn, wg_v[:, a:b], NN)
                uu = _dot(xn, wu_v[:, a:b], NN)
                gu_v[0, rows, a:b] = gg.astype(bf16)
                gu_v[1, rows, a:b] = uu.astype(bf16)
                h_v[rows, a:b] = (gg * uu).astype(bf16)
            return f

        def b_task(a, b):
            def f():
                part_v[rows, a:b] = x_v[rows, a:b].astype(f32) + _dot(h_v[rows, :], wd_v[:, a:b], NN)
            return f

        def do_task():
            bufb_v[i, 0:D, :] = _dot(wop_v[...], dout_v[rows, :], NT)

        def sm_task(gi, lt, sgn):
            def f():
                L = slice(lt * 128, (lt + 1) * 128)
                dst = phq_v if gi < NG else phk_v
                g = gi % NG
                p3 = bufa_v[i, gi * 128:(gi + 1) * 128, L].reshape(DH, 8, 128)
                if sgn == 0:
                    e = jnp.exp(p3 - mm_v[i, 0, gi, :, L][None])
                else:
                    e = jnp.exp(mm_v[i, 1, gi, :, L][None] - p3)
                ph = e * (1.0 / jnp.sum(e, axis=0, keepdims=True))
                dst[i, g * 256 + sgn * 128:g * 256 + (sgn + 1) * 128, L] = ph.reshape(128, 128).astype(bf16)
                if gi >= NG:
                    z_acc[g, sgn * 128:(sgn + 1) * 128, :] += ph.reshape(128, 128)
                fence(ph[DH - 1], (bufa_v,))
            return f

        mx = [gu_task(a, b) for a, b in FBLK] + [do_task, b_task(0, 256), b_task(256, 512)]
        vp = [sm_task(gi, lt, sgn) for gi in range(2 * NG) for lt in range(NLT) for sgn in range(2)]
        _interleave(mx, vp)
        return carry

    _loop("L1", NTL, loop1)

    for g in range(NG):
        kv = _dot(phk_v[0, g * 256:(g + 1) * 256, :], vT_v[0, g * 128:(g + 1) * 128, :], NT)
        for i in range(1, NTL):
            kv = kv + _dot(phk_v[i, g * 256:(g + 1) * 256, :], vT_v[i, g * 128:(g + 1) * 128, :], NT)
        mask_kv = _mask_kv()
        kvm = jnp.where(mask_kv, kv, 0.0)
        kvm_v[g] = kvm.astype(bf16)
        zc = jnp.broadcast_to(jnp.sum(z_acc[g], axis=1, keepdims=True), (256, 128))
        zcol_v[g] = zc
        zm = jnp.where(mask_kv & (_iota((256, 128), 1) < 8), zc, 0.0)
        lhs_v[g, 0:128, :] = kvm.T.astype(bf16)
        lhs_v[g, 128:144, :] = zm.T[0:16, :].astype(bf16)
    for g in range(NG):
        for i in range(NTL):
            bufb_v[i, D + g * 144:D + (g + 1) * 144, :] = _dot(lhs_v[g], phq_v[i, g * 256:(g + 1) * 256, :], NN)

    def loop2(i, carry):
        rows = pl.ds(pl.multiple_of(i * T, T), T)

        def dh_task(a, b):
            def f():
                dh = _dot(dout_v[rows, :], wd_v[a:b, :], NT)
                gq = gu_v[0, rows, a:b].astype(f32)
                uq = gu_v[1, rows, a:b].astype(f32)
                gu_v[0, rows, a:b] = (dh * uq).astype(bf16)
                gu_v[1, rows, a:b] = (dh * gq).astype(bf16)
            return f

        def dxb_task(a, b):
            def f():
                dxb_v[rows, a:b] = (_dot(gu_v[0, rows, :], wg_v[a:b, :], NT)
                                    + _dot(gu_v[1, rows, :], wu_v[a:b, :], NT))
            return f

        def att_task(g, lt):
            def f():
                L = slice(lt * 128, (lt + 1) * 128)
                o0 = D + g * 144
                rden = 1.0 / (bufb_v[i, o0 + 128:o0 + 136, L] + EPS_DEN)
                acc = None
                for hf in range(2):
                    R = slice(hf * 64, (hf + 1) * 64)
                    o3 = bufb_v[i, o0 + hf * 64:o0 + (hf + 1) * 64, L].reshape(8, 8, 128) * rden[None]
                    oT_v[i, g * 128 + hf * 64:g * 128 + (hf + 1) * 64, L] = o3.reshape(64, 128).astype(bf16)
                    do3 = bufb_v[i, g * 128 + hf * 64:g * 128 + (hf + 1) * 64, L].reshape(8, 8, 128)
                    dn_v[i, g * 128 + hf * 64:g * 128 + (hf + 1) * 64, L] = (do3 * rden[None]).reshape(64, 128).astype(bf16)
                    t = jnp.sum(do3 * o3, axis=0)
                    acc = t if acc is None else acc + t
                    fence(acc, (bufb_v,))
                dden = -acc * rden
                dd_v[i, g, :, L] = dden
                fence(dden, (phq_v,))
                for sg in range(2):
                    phq = phq_v[i, g * 256 + sg * 128:g * 256 + (sg + 1) * 128, L].astype(f32)
                    t = phq.reshape(DH, 8, 128) * dden[None]
                    dz_acc[g, sg * 128:(sg + 1) * 128, :] += t.reshape(128, 128)
                    fence(t[DH - 1], (phq_v, bufb_v))
            return f

        mx = [dh_task(a, b) for a, b in FBLK] + [dxb_task(a * 128, (a + 1) * 128) for a in range(4)]
        vp = [att_task(g, lt) for g in range(NG) for lt in range(NLT)]
        _interleave(mx, vp)
        return carry

    _loop("L2", NTL, loop2)

    for g in range(NG):
        dkv = _dot(phq_v[0, g * 256:(g + 1) * 256, :], dn_v[0, g * 128:(g + 1) * 128, :], NT)
        for i in range(1, NTL):
            dkv = dkv + _dot(phq_v[i, g * 256:(g + 1) * 256, :], dn_v[i, g * 128:(g + 1) * 128, :], NT)
        dkvm = jnp.where(_mask_kv(), dkv, 0.0)
        dkvm_v[g] = dkvm.astype(bf16)
        dkvmT_v[g] = dkvm.T.astype(bf16)
        dz_acc[g] = jnp.broadcast_to(jnp.sum(dz_acc[g], axis=1, keepdims=True), (256, 128))
    for g in range(NG):
        for i in range(NTL):
            zt = _tile_lanes(zcol_v[g]).reshape(32, 8, T) * dd_v[i, g][None]
            bufa_v[i, g * 256:(g + 1) * 256, :] = (
                _dot(kvm_v[g], dn_v[i, g * 128:(g + 1) * 128, :], NN) + zt.reshape(256, T))
    for g in range(NG):
        for i in range(NTL):
            bufb_v[i, g * 256:(g + 1) * 256, :] = (
                _dot(dkvm_v[g], vT_v[i, g * 128:(g + 1) * 128, :], NN) + _tile_lanes(dz_acc[g]))
            dyT_v[i, 2 * D + g * 128:2 * D + (g + 1) * 128, :] = _dot(
                dkvmT_v[g], phk_v[i, g * 256:(g + 1) * 256, :], NN).astype(bf16)
    dwo_acc[...] = jnp.zeros(dwo_acc.shape, f32)
    dwd_acc[...] = jnp.zeros(dwd_acc.shape, f32)
    g_acc[...] = jnp.zeros(g_acc.shape, f32)

    def loop3(i, carry):
        rows = pl.ds(pl.multiple_of(i * T, T), T)

        def out_task():
            out_v[rows, :] = (part_v[rows, :] + _dot(oT_v[i], wop_v[...], TN)).astype(bf16)
            pltpu.make_async_copy(out_v.at[rows], out_hbm.at[0, rows], out_sems.at[i]).start()

        def dwo_task():
            dwo_acc[...] += _dot(oT_v[i], dout_v[rows, :], NN)

        def dwd_task(a, b):
            def f():
                dwd_acc[a:b, :] += _dot(h_v[rows, a:b], dout_v[rows, :], TN)
            return f

        def smb_task(gi, lt):
            def f():
                L = slice(lt * 128, (lt + 1) * 128)
                g = gi % NG
                phr = phq_v if gi < NG else phk_v
                dr = bufa_v if gi < NG else bufb_v

                def ld(r0, n):
                    ph = phr[i, g * 256 + r0:g * 256 + r0 + n, L].astype(f32).reshape(n // 8, 8, 128)
                    dp = dr[i, g * 256 + r0:g * 256 + r0 + n, L].reshape(n // 8, 8, 128)
                    return ph, dp

                cs = []
                for sg in range(2):
                    ph, dp = ld(sg * 128, 128)
                    c = jnp.sum(ph * dp, axis=0)
                    cs.append(c)
                    fence(c, (phr, dr))
                NS = 64
                for r0 in range(0, 128, NS):
                    ph0, dp0 = ld(r0, NS)
                    ph1, dp1 = ld(128 + r0, NS)
                    d = ph0 * (dp0 - cs[0][None]) - ph1 * (dp1 - cs[1][None])
                    dyT_v[i, gi * 128 + r0:gi * 128 + r0 + NS, L] = d.reshape(NS, 128).astype(bf16)
                    fence(d[NS // 8 - 1], (phq_v, bufa_v, phk_v, bufb_v))
            return f

        mx = [dwo_task, out_task] + [dwd_task(a * 256, (a + 1) * 256) for a in range(7)]
        vp = [smb_task(gi, lt) for gi in range(2 * NG) for lt in range(NLT)]
        _interleave(mx, vp)
        return carry

    _loop("L3", NTL, loop3)
    base = NTL
    dwd_v[...] = dwd_acc[...].astype(bf16)
    c_dwd = pltpu.make_async_copy(dwd_v, dwd_hbm, out_sems.at[base + 3])
    c_dwd.start()
    for g in range(NG):
        dwo_v[g * 128:(g + 1) * 128, :] = _dot(_pmT(), dwo_acc[g * 128:(g + 1) * 128, :].astype(bf16), NN).astype(bf16)
    c_dwo = pltpu.make_async_copy(dwo_v, dwo_hbm, out_sems.at[base + 2])
    c_dwo.start()

    def loop4(c, carry):
        g_acc[...] += _dot(xnT_v[2 * c], dyT_v[2 * c], NT) + _dot(xnT_v[2 * c + 1], dyT_v[2 * c + 1], NT)
        for s in range(2):
            i = c * 2 + s
            rows = pl.ds(pl.multiple_of(i * T, T), T)
            dxb_v[rows, :] += _dot(dyT_v[i], wpT_v[...], TN)
        return carry

    _loop("L4", NTL // 2, loop4)

    def lnb_tile(i):
        RC = 32
        for s in range(T // RC):
            rows = pl.ds(pl.multiple_of(i * T + s * RC, RC), RC)
            dxn = dxb_v[rows, :]
            rstd = rstd_v[rows, :]
            xn = (x_v[rows, :].astype(f32) - mean_v[rows, :]) * rstd
            m1 = jnp.mean(dxn, axis=1, keepdims=True)
            m2 = jnp.mean(dxn * xn, axis=1, keepdims=True)
            dx = (dxn - m1 - xn * m2) * rstd
            gx_v[rows, :] = (dout_v[rows, :].astype(f32) + dx).astype(bf16)
        rows = pl.ds(pl.multiple_of(i * T, T), T)
        pltpu.make_async_copy(gx_v.at[rows], gx_hbm.at[0, rows], out_sems.at[base + 4 + i]).start()

    mphi_l = (_iota((128, 128), 1) % 8) == (_iota((128, 128), 0) // DH)
    mgs = []
    for g in range(NG):
        ph_g = phi_v[g * 128:(g + 1) * 128, :]
        gq = g_acc[:, g * 128:(g + 1) * 128].astype(bf16)
        gk = g_acc[:, D + g * 128:D + (g + 1) * 128].astype(bf16)
        gv = g_acc[:, 2 * D + g * 128:2 * D + (g + 1) * 128].astype(bf16)
        dwqkv_v[:, g * 128:(g + 1) * 128] = _dot(gq, ph_g, NT).astype(bf16)
        dwqkv_v[:, D + g * 128:D + (g + 1) * 128] = _dot(gk, ph_g, NT).astype(bf16)
        dwqkv_v[:, 2 * D + g * 128:2 * D + (g + 1) * 128] = _dot(gv, _pm(), NN).astype(bf16)
        mg = (_dot(wqkv_v[:, g * 128:(g + 1) * 128], gq, TN)
              + _dot(wqkv_v[:, D + g * 128:D + (g + 1) * 128], gk, TN))
        mgs.append(jnp.where(mphi_l, mg, 0.0).astype(bf16))
    mm = jnp.concatenate(mgs, axis=0)
    ym = jnp.where(_mask_d(), _dot(mm, _e2(), NT), 0.0).astype(bf16)
    dwphi_v[...] = _dot(ym, _lh(), TN).astype(bf16).reshape(DH, DH, H)
    c_dwqkv = pltpu.make_async_copy(dwqkv_v, dwqkv_hbm, out_sems.at[base])
    c_dwqkv.start()
    c_dwphi = pltpu.make_async_copy(dwphi_v, dwphi_hbm, out_sems.at[base + 1])
    c_dwphi.start()
    lnb_tile(NTL - 1)

    NB5 = 7
    FB5 = F // NB5

    def loop5(j, carry):
        cols = pl.ds(pl.multiple_of(j * FB5, FB5), FB5)
        lnb_tile(j)
        for k, (dst_v, dst_hbm) in enumerate(((dwg_v, dwg_hbm), (dwu_v, dwu_hbm))):
            acc = _dot(xnT_v[0], gu_v[k, 0:T, cols], NN)
            for i in range(1, NTL):
                acc = acc + _dot(xnT_v[i], gu_v[k, i * T:(i + 1) * T, cols], NN)
            dst_v[:, cols] = acc.astype(bf16)
            pltpu.make_async_copy(dst_v.at[:, cols], dst_hbm.at[:, cols], out_sems.at[base + 12 + k * NB5 + j]).start()
        return carry

    _loop("L5", NB5, loop5)

    for i in range(NTL):
        rows = pl.ds(i * T, T)
        pltpu.make_async_copy(out_v.at[rows], out_hbm.at[0, rows], out_sems.at[i]).wait()
        pltpu.make_async_copy(gx_v.at[rows], gx_hbm.at[0, rows], out_sems.at[base + 4 + i]).wait()
    c_dwqkv.wait()
    c_dwphi.wait()
    c_dwo.wait()
    c_dwd.wait()
    for k, (dst_v, dst_hbm) in enumerate(((dwg_v, dwg_hbm), (dwu_v, dwu_hbm))):
        for j in range(NB5):
            cols = pl.ds(j * FB5, FB5)
            pltpu.make_async_copy(dst_v.at[:, cols], dst_hbm.at[:, cols], out_sems.at[base + 12 + k * NB5 + j]).wait()


@jax.jit
def pallas_parallel_sum__linear_kernel_hedgehog__glu_gated_bilinear__prompt_kernel(
    A_x: jax.Array,
    A_wqkv: jax.Array,
    A_w_phi: jax.Array,
    A_wo: jax.Array,
    B_x: jax.Array,
    B_w_gate: jax.Array,
    B_w_up: jax.Array,
    B_w_down: jax.Array,
    grad_out: jax.Array,
):
    del B_x
    V = pltpu.VMEM
    n_out_sems = NTL + 12 + 14
    scratch = [
        V((S, D), bf16), V((D, 3 * D), bf16), V((DH, DH, H), bf16), V((D, D), bf16),
        V((D, F), bf16), V((D, F), bf16), V((F, D), bf16), V((S, D), bf16),
        V((3 * D, D), bf16), V((D, D), bf16), V((D, 128), bf16),
        V((S, D), bf16), V((NTL, D, T), bf16), V((S, 1), f32), V((S, 1), f32),
        V((NTL + 1, 2 * D, T), f32), V((NTL + 1, D + NG * 144, T), f32), V((NTL, 2, 2 * NG, 8, T), f32),
        V((NTL + 1, 2 * D, T), bf16), V((NTL + 1, 2 * D, T), bf16), V((NTL, D, T), bf16),
        V((2, S, F), bf16), V((S, F), bf16), V((S, D), f32), V((S, D), f32),
        V((NG, 256, 128), f32), V((NG, 144, 256), bf16),
        V((NG, 256, 128), bf16), V((NG, 256, 128), f32),
        V((NTL, D, T), bf16), V((NTL, 3 * D, T), bf16), V((NTL, D, T), bf16), V((NTL, NG, 8, T), f32),
        V((NG, 256, 128), f32), V((NG, 256, 128), bf16), V((NG, 128, 256), bf16),
        V((D, 3 * D), f32), V((D, D), f32), V((F, D), f32),
        V((S, D), bf16), V((S, D), bf16), V((D, 3 * D), bf16), V((DH, DH, H), bf16),
        V((D, D), bf16), V((D, F), bf16), V((D, F), bf16), V((F, D), bf16),
        pltpu.SMEM((1,), jnp.int32),
        pltpu.SemaphoreType.DMA((7,)), pltpu.SemaphoreType.DMA((NC0,)), pltpu.SemaphoreType.DMA((n_out_sems,)),
    ]
    out_shape = (
        jax.ShapeDtypeStruct((1, S, D), bf16),
        jax.ShapeDtypeStruct((1, S, D), bf16),
        jax.ShapeDtypeStruct((D, 3 * D), bf16),
        jax.ShapeDtypeStruct((DH, DH, H), bf16),
        jax.ShapeDtypeStruct((D, D), bf16),
        jax.ShapeDtypeStruct((D, F), bf16),
        jax.ShapeDtypeStruct((D, F), bf16),
        jax.ShapeDtypeStruct((F, D), bf16),
    )
    any_spec = pl.BlockSpec(memory_space=pl.ANY)
    outs = pl.pallas_call(
        _kernel,
        out_shape=out_shape,
        in_specs=[any_spec] * 8,
        out_specs=tuple([any_spec] * 8),
        scratch_shapes=scratch,
        compiler_params=pltpu.CompilerParams(vmem_limit_bytes=120 * 1024 * 1024),
    )(A_x, A_wqkv, jnp.transpose(A_w_phi, (1, 2, 0)), A_wo, B_w_gate, B_w_up, B_w_down, grad_out)
    out, gx, dwqkv, dwphi_t, dwo, dwg, dwu, dwd = outs
    return (out, gx, dwqkv, jnp.transpose(dwphi_t, (2, 0, 1)), dwo, dwg, dwu, dwd)
```

```python
import jax
import jax.numpy as jnp
from jax import lax
import jax.experimental.pallas as pl
import jax.experimental.pallas.tpu as pltpu

S, D, F, H, DH = 2048, 512, 1792, 32, 16
NG = 4
NT4 = 8
NDR = 64
T = 512
NTL = S // T
NLT = T // 128
EPS_LN = 1e-5
EPS_DEN = 1e-6

f32, bf16 = jnp.float32, jnp.bfloat16
NN = (((1,), (0,)), ((), ()))
NT = (((1,), (1,)), ((), ()))
TN = (((0,), (0,)), ((), ()))
TT = (((0,), (1,)), ((), ()))


def _dot(a, b, dn):
    return lax.dot_general(a, b, dn, preferred_element_type=f32)


def _iota(shape, dim):
    return lax.broadcasted_iota(jnp.int32, shape, dim)


def _onehot(cond):
    return jnp.where(cond, 1.0, 0.0).astype(bf16)


def _hl(r):
    return (r // 64) * 4 + r % 4


def _ff(r):
    return ((r // 4) % 2) * 8 + (r // 8) % 8


def _mask4(shape, rows_per_head):
    return (_iota(shape, 0) // rows_per_head) == (_iota(shape, 1) % 4)


def _fold4(a, op):
    return op(a, pltpu.roll(a, 4, 0))


def _lh():
    return _onehot(_iota((D, H), 0) // DH == _iota((D, H), 1))


def _mask_d():
    return (_iota((D, 256), 0) % DH) == (_iota((D, 256), 1) // DH)


def _e2():
    return _onehot(_iota((256, 128), 0) % DH == _ff(_iota((256, 128), 1)))


def _wide(a):
    return jnp.concatenate([a] * 4, axis=1)


def _fold_lanes(a):
    return (a[:, 0:128] + a[:, 128:256]) + (a[:, 256:384] + a[:, 384:512])


def _row_mean(ps):
    return jnp.broadcast_to(jnp.sum(ps, axis=1, keepdims=True) * (1.0 / D), ps.shape)


def _interleave(mxu_tasks, vpu_tasks):
    nm, nv = len(mxu_tasks), len(vpu_tasks)
    done = 0
    for k, task in enumerate(mxu_tasks):
        task()
        if k < nm - 1:
            upto = min((nv * (k + 1) + nm - 2) // (nm - 1), nv)
            while done < upto:
                vpu_tasks[done]()
                done += 1
    assert done == nv


def _kernel(x_hbm, wqkv_hbm, wphi_hbm, wo_hbm, wg_hbm, wu_hbm, wd_hbm, dout_hbm,
            out_hbm, gx_hbm, dwqkv_hbm, dwphi_hbm, dwo_hbm, dwg_hbm, dwu_hbm, dwd_hbm,
            x_v, wqkv_v, wphi_v, wo_v, wg_v, wu_v, wd_v, dout_v,
            wpT_v, phi_v,
            xn_v, xnT_v, mean_v, rstd_v,
            bufa_v, bufb_v, mm_v, phq_v, phk_v, vT_v,
            gu_v, h_v, part_v, dxb_v,
            z_acc, lhs_v, kvm_v, zcol_v,
            oT_v, dyT_v, dn_v, dd_v,
            dz_acc, dkvm_v, dkvmT_v,
            g_acc, dwo_acc, dwd_acc,
            out_v, gx_v, dwqkv_v, dwphi_v, dwo_v, dwg_v, dwu_v, dwd_v,
            pad_s, in_sems, x_sems, out_sems):
    def tile_rows(c):
        return pl.ds(pl.multiple_of(c * T, T), T)

    def cp_x(c):
        return pltpu.make_async_copy(x_hbm.at[0, tile_rows(c)], x_v.at[tile_rows(c)], x_sems.at[c])

    def cp_do(c):
        return pltpu.make_async_copy(dout_hbm.at[0, tile_rows(c)], dout_v.at[tile_rows(c)], x_sems.at[NTL + c])

    cp_wqkv = pltpu.make_async_copy(wqkv_hbm, wqkv_v, in_sems.at[0])
    cp_wphi = pltpu.make_async_copy(wphi_hbm, wphi_v, in_sems.at[1])
    cp_wg = pltpu.make_async_copy(wg_hbm, wg_v, in_sems.at[2])
    cp_wu = pltpu.make_async_copy(wu_hbm, wu_v, in_sems.at[3])
    cp_wo = pltpu.make_async_copy(wo_hbm, wo_v, in_sems.at[4])
    WDP = ((0, 512), (512, 1280), (1280, 1792))
    cp_wd = [pltpu.make_async_copy(wd_hbm.at[pl.ds(a, b - a)], wd_v.at[pl.ds(a, b - a)], in_sems.at[5 + k])
             for k, (a, b) in enumerate(WDP)]
    cp_wphi.start()
    cp_wd[0].start()
    cp_do(0).start()
    cp_wd[1].start()

    pad_s[0] = 2 * D
    pad_s[1] = S
    pad_s[2] = D + NT4 * NDR
    pad_s[3] = 3 * D
    z_acc[...] = jnp.zeros(z_acc.shape, f32)
    dz_acc[...] = jnp.zeros(dz_acc.shape, f32)

    def fence(v, refs):
        for r in refs:
            pad = pl.multiple_of(pad_s[2] if r is bufb_v else pad_s[0], 16)
            if r.dtype == bf16:
                r[0, pl.ds(pad, 16), 0:128] = jnp.concatenate([v, v], axis=0).astype(bf16)
            else:
                r[0, pl.ds(pad, 8), 0:128] = v

    def xfence(v):
        x_v[pl.ds(pl.multiple_of(pad_s[1], 16), 16), 0:128] = v[0:16, 0:128].astype(bf16)

    def ln_tile_bg(c):
        RC = 32
        for s in range(T // RC):
            rows = pl.ds(pl.multiple_of(c * T + s * RC, RC), RC)
            x = x_v[rows, :].astype(f32)
            m = _row_mean(_fold_lanes(x))
            xc = x - _wide(m)
            rstd = lax.rsqrt(_row_mean(_fold_lanes(xc * xc)) + EPS_LN)
            mean_v[rows, :] = m
            rstd_v[rows, :] = rstd
            xn = xc * _wide(rstd)
            xn_v[rows, :] = xn.astype(bf16)
            if s % 2 == 1:
                xfence(xn)

    def dh_cols(rows, a, b):
        for c0 in range(a, b, 256):
            gu_v[1, rows, c0:c0 + 256] = _dot(dout_v[rows, :], wd_v[c0:c0 + 256, :], NT).astype(bf16)

    cp_wphi.wait()
    wt = wphi_v[...].reshape(256, H)
    bmat = jnp.where(_mask_d(), _dot(_lh(), wt, NT), 0.0).astype(bf16)
    mask_h = _hl(_iota((D, 128), 1)) == ((_iota((D, 128), 0) // DH) % 8)
    phi_v[...] = jnp.where(mask_h, _dot(bmat, _e2(), NN), 0.0).astype(bf16)
    cp_wd[0].wait()
    cp_do(0).wait()
    cp_wd[2].start()
    cp_do(1).start()
    dh_cols(pl.ds(0, T), *WDP[0])
    cp_wd[1].wait()
    cp_x(0).start()
    dh_cols(pl.ds(0, T), *WDP[1])
    cp_wd[2].wait()
    cp_do(2).start()
    cp_x(1).start()
    cp_do(3).start()
    cp_x(2).start()
    dh_cols(pl.ds(0, T), *WDP[2])

    def loopa(j, carry):
        cp_do(j + 1).wait()
        cp_x(j).wait()

        @pl.when(j == 0)
        def _():
            cp_wqkv.start()
            cp_x(3).start()
            cp_wo.start()

        @pl.when(j == 1)
        def _():
            cp_wg.start()
            cp_wu.start()

        dh_cols(tile_rows(j + 1), 0, F)
        ln_tile_bg(j)
        return carry

    lax.fori_loop(0, NTL - 1, loopa, 0)

    cp_wqkv.wait()
    cp_x(3).wait()
    cp_wo.wait()
    wpT_v[2 * D:3 * D, :] = wqkv_v[:, 2 * D:3 * D].T
    for g in range(NG):
        ph_g = phi_v[g * 128:(g + 1) * 128, :]
        wq_g = wqkv_v[:, g * 128:(g + 1) * 128]
        wk_g = wqkv_v[:, D + g * 128:D + (g + 1) * 128]
        wpT_v[g * 128:(g + 1) * 128, :] = _dot(ph_g, wq_g, TT).astype(bf16)
        wpT_v[D + g * 128:D + (g + 1) * 128, :] = _dot(ph_g, wk_g, TT).astype(bf16)

    def loop0(c, carry):
        pT = _dot(wpT_v[0:3 * D, :], xn_v[tile_rows(c), :], NT)
        p = pT[0:2 * D]
        bufa_v[c, 0:2 * D, :] = p
        p4 = p.reshape(2 * NT4, 8, 8, T)
        mxs = jnp.max(p4, axis=1)
        mns = jnp.min(p4, axis=1)
        for ti in range(2 * NT4):
            mm_v[c, 0, ti] = _fold4(mxs[ti], jnp.maximum)
            mm_v[c, 1, ti] = _fold4(mns[ti], jnp.minimum)
        vT_v[c] = pT[2 * D:3 * D].astype(bf16)
        ln_tile_bg(NTL - 1)
        bufb_v[c, 0:D, :] = _dot(wo_v[...], dout_v[tile_rows(c), :], NT)
        return carry

    lax.fori_loop(0, NTL, loop0, 0)
    cp_wg.wait()
    cp_wu.wait()

    def dwd_task(rows, a, b):
        def f():
            dwd_acc[a:b, :] += _dot(h_v[rows, a:b], dout_v[rows, :], TN)
        return f

    def loop1(i, carry):
        rows = tile_rows(i)

        def gu_task(a, b):
            def f():
                xn = xn_v[rows, :]
                gg = _dot(xn, wg_v[:, a:b], NN)
                uu = _dot(xn, wu_v[:, a:b], NN)
                dh = gu_v[1, rows, a:b].astype(f32)
                gu_v[0, rows, a:b] = (dh * uu).astype(bf16)
                gu_v[1, rows, a:b] = (dh * gg).astype(bf16)
                h_v[rows, a:b] = (gg * uu).astype(bf16)
            return f

        def sm_task(ti, lt):
            def f():
                L = slice(lt * 128, (lt + 1) * 128)
                dst = phq_v if ti < NT4 else phk_v
                t4 = ti % NT4
                p3 = bufa_v[i, ti * 64:(ti + 1) * 64, L].reshape(8, 8, 128)
                for sgn in range(2):
                    if sgn == 0:
                        e = jnp.exp(p3 - mm_v[i, 0, ti, :, L][None])
                    else:
                        e = jnp.exp(mm_v[i, 1, ti, :, L][None] - p3)
                    ph = e * (1.0 / _fold4(jnp.sum(e, axis=0), jnp.add))[None]
                    dst[i, t4 * 128 + sgn * 64:t4 * 128 + (sgn + 1) * 64, L] = ph.reshape(64, 128).astype(bf16)
                    if ti >= NT4:
                        z_acc[t4, sgn * 64:(sgn + 1) * 64, :] += ph.reshape(64, 128)
                fence(ph[7], (bufa_v,))
            return f

        mx = [gu_task(a * 256, (a + 1) * 256) for a in range(7)]
        vp = [sm_task(ti, lt) for ti in range(2 * NT4) for lt in range(NLT)]
        _interleave(mx, vp)
        return carry

    lax.fori_loop(0, NTL, loop1, 0)

    def pair_lhs(a, b):
        zero = jnp.zeros((64, 128), f32)
        xm = jnp.concatenate([jnp.concatenate([a, zero], axis=1), jnp.concatenate([zero, b], axis=1)], axis=0)
        return xm.T.astype(bf16)

    kvs = []
    for t4 in range(NT4):
        kv = _dot(vT_v[0, t4 * 64:(t4 + 1) * 64, :], phk_v[0, t4 * 128:(t4 + 1) * 128, :], NT)
        for i in range(1, NTL):
            kv = kv + _dot(vT_v[i, t4 * 64:(t4 + 1) * 64, :], phk_v[i, t4 * 128:(t4 + 1) * 128, :], NT)
        kvm = jnp.where(_mask4((64, 128), DH), kv, 0.0)
        kvs.append(kvm)
        zcol_v[t4] = jnp.broadcast_to(jnp.sum(z_acc[t4], axis=1, keepdims=True), (128, 128))
        lhs_v[t4] = kvm.astype(bf16)
    for j in range(NG):
        kvm_v[j] = pair_lhs(kvs[2 * j], kvs[2 * j + 1])
    for t4 in range(NT4):
        for i in range(NTL):
            bufb_v[i, D + t4 * NDR:D + (t4 + 1) * NDR, :] = _dot(lhs_v[t4], phq_v[i, t4 * 128:(t4 + 1) * 128, :], NN)

    def loop2(i, carry):
        rows = tile_rows(i)

        def b_task(a, b):
            def f():
                part_v[rows, a:b] = x_v[rows, a:b].astype(f32) + _dot(h_v[rows, :], wd_v[:, a:b], NN)
            return f

        def dxb_task(a, b):
            def f():
                dxb_v[rows, a:b] = (_dot(gu_v[0, rows, :], wg_v[a:b, :], NT)
                                    + _dot(gu_v[1, rows, :], wu_v[a:b, :], NT))
            return f

        def att_task(t4, lt):
            def f():
                L = slice(lt * 128, (lt + 1) * 128)
                o0 = D + t4 * NDR
                sub = _iota((8, 128), 0)
                den = None
                for sg in range(2):
                    R = slice(t4 * 128 + sg * 64, t4 * 128 + (sg + 1) * 64)
                    t = phq_v[i, R, L].astype(f32) * zcol_v[t4, sg * 64:(sg + 1) * 64, :]
                    t = jnp.sum(t.reshape(8, 8, 128), axis=0)
                    den = t if den is None else den + t
                    fence(den, (phq_v,))
                rd = 1.0 / (_fold4(den, jnp.add) + EPS_DEN)
                fence(rd, (bufb_v,))
                aa = []
                for hp in range(2):
                    R = slice(t4 * 64 + hp * 32, t4 * 64 + (hp + 1) * 32)
                    rden = jnp.stack([jnp.broadcast_to(rd[2 * hp + k:2 * hp + k + 1, :], (8, 128)) for k in range(2)])[:, None]
                    o4 = bufb_v[i, o0 + hp * 32:o0 + (hp + 1) * 32, L].reshape(2, 2, 8, 128) * rden
                    oT_v[i, R, L] = o4.reshape(32, 128).astype(bf16)
                    do4 = bufb_v[i, R, L].reshape(2, 2, 8, 128)
                    dn_v[i, R, L] = (do4 * rden).reshape(32, 128).astype(bf16)
                    tt = jnp.sum(do4 * o4, axis=1) * rden[:, 0]
                    aa.append(jnp.where(sub % 2 == 0, tt[0] + pltpu.roll(tt[0], 7, 0), tt[1] + pltpu.roll(tt[1], 1, 0)))
                    fence(tt[1], (bufb_v,))
                a = jnp.where(sub % 4 < 2, aa[0] + pltpu.roll(aa[0], 6, 0), aa[1] + pltpu.roll(aa[1], 2, 0))
                dden = -_fold4(a, jnp.add)
                dd_v[i, t4, :, L] = dden
                fence(dden, (phq_v,))
                for sg in range(2):
                    phq = phq_v[i, t4 * 128 + sg * 64:t4 * 128 + (sg + 1) * 64, L].astype(f32)
                    t = phq.reshape(8, 8, 128) * dden[None]
                    dz_acc[t4, sg * 64:(sg + 1) * 64, :] += t.reshape(64, 128)
                    fence(t[7], (phq_v, bufb_v))
            return f

        mx = [dxb_task(a * 128, (a + 1) * 128) for a in range(4)] + [b_task(0, 256), b_task(256, 512)]
        vp = [att_task(t4, lt) for t4 in range(NT4) for lt in range(NLT)]
        _interleave(mx, vp)
        return carry

    lax.fori_loop(0, NTL, loop2, 0)

    dkvs = []
    for t4 in range(NT4):
        dkv = _dot(dn_v[0, t4 * 64:(t4 + 1) * 64, :], phq_v[0, t4 * 128:(t4 + 1) * 128, :], NT)
        for i in range(1, NTL):
            dkv = dkv + _dot(dn_v[i, t4 * 64:(t4 + 1) * 64, :], phq_v[i, t4 * 128:(t4 + 1) * 128, :], NT)
        dkvm = jnp.where(_mask4((64, 128), DH), dkv, 0.0)
        dkvs.append(dkvm)
        dkvmT_v[t4] = dkvm.astype(bf16)
        dz_acc[t4] = jnp.broadcast_to(jnp.sum(dz_acc[t4], axis=1, keepdims=True), (128, 128))
    for j in range(NG):
        dkvm_v[j] = pair_lhs(dkvs[2 * j], dkvs[2 * j + 1])
    for j in range(NG):
        for i in range(NTL):
            r = _dot(kvm_v[j], dn_v[i, j * 128:(j + 1) * 128, :], NN)
            for t2 in range(2):
                t4 = 2 * j + t2
                zt = _wide(zcol_v[t4]).reshape(16, 8, T) * dd_v[i, t4][None]
                bufa_v[i, t4 * 128:(t4 + 1) * 128, :] = r[t2 * 128:(t2 + 1) * 128] + zt.reshape(128, T)
    for j in range(NG):
        for i in range(NTL):
            r = _dot(dkvm_v[j], vT_v[i, j * 128:(j + 1) * 128, :], NN)
            for t2 in range(2):
                t4 = 2 * j + t2
                bufb_v[i, t4 * 128:(t4 + 1) * 128, :] = r[t2 * 128:(t2 + 1) * 128] + _wide(dz_acc[t4])
                dyT_v[i, 2 * D + t4 * 64:2 * D + (t4 + 1) * 64, :] = _dot(
                    dkvmT_v[t4], phk_v[i, t4 * 128:(t4 + 1) * 128, :], NN).astype(bf16)
    dwo_acc[...] = jnp.zeros(dwo_acc.shape, f32)
    dwd_acc[...] = jnp.zeros(dwd_acc.shape, f32)
    g_acc[...] = jnp.zeros(g_acc.shape, f32)

    def loop3(i, carry):
        rows = tile_rows(i)

        def out_task():
            out_v[rows, :] = (part_v[rows, :] + _dot(oT_v[i], wo_v[...], TN)).astype(bf16)
            pltpu.make_async_copy(out_v.at[rows], out_hbm.at[0, rows], out_sems.at[0]).start()

        def dwo_task():
            dwo_acc[...] += _dot(oT_v[i], dout_v[rows, :], NN)

        def smb_task(ti, lt):
            def f():
                L = slice(lt * 128, (lt + 1) * 128)
                t4 = ti % NT4
                phr = phq_v if ti < NT4 else phk_v
                dr = bufa_v if ti < NT4 else bufb_v
                ds = []
                for sg in range(2):
                    r0 = t4 * 128 + sg * 64
                    ph = phr[i, r0:r0 + 64, L].astype(f32).reshape(8, 8, 128)
                    dp = dr[i, r0:r0 + 64, L].reshape(8, 8, 128)
                    c = _fold4(jnp.sum(ph * dp, axis=0), jnp.add)
                    ds.append(ph * (dp - c[None]))
                    if sg == 0:
                        fence(ds[0][7], (phr, dr))
                d = ds[0] - ds[1]
                dyT_v[i, ti * 64:(ti + 1) * 64, L] = d.reshape(64, 128).astype(bf16)
                fence(d[7], (phq_v, bufa_v, phk_v, bufb_v))
            return f

        mx = [dwo_task, out_task] + [dwd_task(rows, a * 256, (a + 1) * 256) for a in range(7)]
        def xt_task():
            xnT_v[i] = xn_v[rows, :].T

        vp = [xt_task] + [smb_task(ti, lt) for ti in range(2 * NT4) for lt in range(NLT)]
        _interleave(mx, vp)
        return carry

    lax.fori_loop(0, NTL, loop3, 0)

    def lnb_rows(r0, nsub):
        RC = 32
        for s in range(nsub):
            rows = pl.ds(pl.multiple_of(r0 + s * RC, RC), RC)
            dxn = dxb_v[rows, :]
            rstd = rstd_v[rows, 0:1]
            xn = (x_v[rows, :].astype(f32) - mean_v[rows, 0:1]) * rstd
            m1 = jnp.mean(dxn, axis=1, keepdims=True)
            m2 = jnp.mean(dxn * xn, axis=1, keepdims=True)
            dx = (dxn - m1 - xn * m2) * rstd
            gx_v[rows, :] = (dout_v[rows, :].astype(f32) + dx).astype(bf16)
        rows = pl.ds(pl.multiple_of(r0, RC), RC * nsub)
        pltpu.make_async_copy(gx_v.at[rows], gx_hbm.at[0, rows], out_sems.at[1]).start()

    def loop4(i, carry):
        g_acc[...] += _dot(xnT_v[i], dyT_v[i], NT)
        fr = pl.ds(pl.multiple_of(i * (F // 4), F // 4), F // 4)
        dwd_v[fr, :] = dwd_acc[fr, :].astype(bf16)
        pltpu.make_async_copy(dwd_v.at[fr], dwd_hbm.at[fr], out_sems.at[5]).start()
        orr = pl.ds(pl.multiple_of(i * (D // 4), D // 4), D // 4)
        dwo_v[orr, :] = dwo_acc[orr, :].astype(bf16)
        pltpu.make_async_copy(dwo_v.at[orr], dwo_hbm.at[orr], out_sems.at[4]).start()
        last = pl.ds(pl.multiple_of(i * (F // 4) + F // 4 - 16, 16), 16)
        lasto = pl.ds(pl.multiple_of(i * (D // 4) + D // 4 - 16, 16), 16)
        wpad = pl.ds(pl.multiple_of(pad_s[3], 16), 16)
        wpT_v[wpad, 0:128] = dwd_v[last, D - 128:D]
        wpT_v[wpad, 128:256] = dwo_v[lasto, D - 128:D]
        dxb_v[tile_rows(i), :] += _dot(dyT_v[i], wpT_v[0:3 * D, :], TN)
        return carry

    lax.fori_loop(0, NTL, loop4, 0)

    lnb_rows(S - 32, 1)

    def dwqk(g):
        ph_g = phi_v[g * 128:(g + 1) * 128, :]
        gq = g_acc[:, g * 128:(g + 1) * 128].astype(bf16)
        gk = g_acc[:, D + g * 128:D + (g + 1) * 128].astype(bf16)
        dwqkv_v[:, g * 128:(g + 1) * 128] = _dot(gq, ph_g, NT).astype(bf16)
        dwqkv_v[:, D + g * 128:D + (g + 1) * 128] = _dot(gk, ph_g, NT).astype(bf16)

    mphi_l = _hl(_iota((128, 128), 1)) == (_iota((128, 128), 0) // DH)
    mgs = []
    for g in range(NG):
        gq = g_acc[:, g * 128:(g + 1) * 128].astype(bf16)
        gk = g_acc[:, D + g * 128:D + (g + 1) * 128].astype(bf16)
        mg = (_dot(wqkv_v[:, g * 128:(g + 1) * 128], gq, TN)
              + _dot(wqkv_v[:, D + g * 128:D + (g + 1) * 128], gk, TN))
        mgs.append(jnp.where(mphi_l, mg, 0.0).astype(bf16))
    vcols = pl.ds(2 * D, D)
    dwqkv_v[:, 2 * D:3 * D] = g_acc[:, 2 * D:3 * D].astype(bf16)
    pltpu.make_async_copy(dwqkv_v.at[:, vcols], dwqkv_hbm.at[:, vcols], out_sems.at[2]).start()
    dwqk(0)
    dwqk(1)
    mm = jnp.concatenate(mgs, axis=0)
    ym = jnp.where(_mask_d(), _dot(mm, _e2(), NT), 0.0).astype(bf16)
    dwqk(2)
    dwqk(3)
    qkcols = pl.ds(0, 2 * D)
    pltpu.make_async_copy(dwqkv_v.at[:, qkcols], dwqkv_hbm.at[:, qkcols], out_sems.at[2]).start()
    dwphi_v[...] = _dot(ym, _lh(), TN).astype(bf16).reshape(DH, DH, H)
    c_dwphi = pltpu.make_async_copy(dwphi_v, dwphi_hbm, out_sems.at[3])
    c_dwphi.start()

    NB5 = 7
    FB5 = F // NB5

    def loop5(j, carry):
        lnb_rows(j * 288, 9)
        for k, off, width in ((0, 0, FB5), (1, 0, FB5 // 2), (1, FB5 // 2, FB5 // 2)):
            dst_v, dst_hbm = ((dwg_v, dwg_hbm), (dwu_v, dwu_hbm))[k]
            cols = pl.ds(pl.multiple_of(j * FB5 + off, 128), width)
            acc = _dot(xnT_v[0], gu_v[k, 0:T, cols], NN)
            for i in range(1, NTL):
                acc = acc + _dot(xnT_v[i], gu_v[k, i * T:(i + 1) * T, cols], NN)
            dst_v[:, cols] = acc.astype(bf16)
            pltpu.make_async_copy(dst_v.at[:, cols], dst_hbm.at[:, cols], out_sems.at[6 + k]).start()
        return carry

    lax.fori_loop(0, NB5, loop5, 0)

    pltpu.make_async_copy(out_v, out_hbm.at[0], out_sems.at[0]).wait()
    pltpu.make_async_copy(dwqkv_v, dwqkv_hbm, out_sems.at[2]).wait()
    c_dwphi.wait()
    pltpu.make_async_copy(dwo_v, dwo_hbm, out_sems.at[4]).wait()
    pltpu.make_async_copy(dwd_v, dwd_hbm, out_sems.at[5]).wait()
    pltpu.make_async_copy(gx_v, gx_hbm.at[0], out_sems.at[1]).wait()
    pltpu.make_async_copy(dwg_v, dwg_hbm, out_sems.at[6]).wait()
    pltpu.make_async_copy(dwu_v, dwu_hbm, out_sems.at[7]).wait()


@jax.jit
def pallas_parallel_sum__linear_kernel_hedgehog__glu_gated_bilinear__prompt_kernel(
    A_x: jax.Array,
    A_wqkv: jax.Array,
    A_w_phi: jax.Array,
    A_wo: jax.Array,
    B_x: jax.Array,
    B_w_gate: jax.Array,
    B_w_up: jax.Array,
    B_w_down: jax.Array,
    grad_out: jax.Array,
):
    del B_x
    V = pltpu.VMEM
    scratch = [
        V((S + 16, D), bf16), V((D, 3 * D), bf16), V((DH, DH, H), bf16), V((D, D), bf16),
        V((D, F), bf16), V((D, F), bf16), V((F, D), bf16), V((S, D), bf16),
        V((3 * D + 16, D), bf16), V((D, 128), bf16),
        V((S, D), bf16), V((NTL, D, T), bf16), V((S, 128), f32), V((S, 128), f32),
        V((NTL, 2 * D + 16, T), f32), V((NTL, D + NT4 * NDR + 16, T), f32), V((NTL, 2, 2 * NT4, 8, T), f32),
        V((NTL, 2 * D + 16, T), bf16), V((NTL, 2 * D + 16, T), bf16), V((NTL, D, T), bf16),
        V((2, S, F), bf16), V((S, F), bf16), V((S, D), f32), V((S, D), f32),
        V((NT4, 128, 128), f32), V((NT4, NDR, 128), bf16),
        V((NG, 256, 128), bf16), V((NT4, 128, 128), f32),
        V((NTL, D, T), bf16), V((NTL, 3 * D, T), bf16), V((NTL, D, T), bf16), V((NTL, NT4, 8, T), f32),
        V((NT4, 128, 128), f32), V((NG, 256, 128), bf16), V((NT4, 64, 128), bf16),
        V((D, 3 * D), f32), V((D, D), f32), V((F, D), f32),
        V((S, D), bf16), V((S, D), bf16), V((D, 3 * D), bf16), V((DH, DH, H), bf16),
        V((D, D), bf16), V((D, F), bf16), V((D, F), bf16), V((F, D), bf16),
        pltpu.SMEM((4,), jnp.int32),
        pltpu.SemaphoreType.DMA((8,)), pltpu.SemaphoreType.DMA((2 * NTL,)), pltpu.SemaphoreType.DMA((8,)),
    ]
    out_shape = (
        jax.ShapeDtypeStruct((1, S, D), bf16),
        jax.ShapeDtypeStruct((1, S, D), bf16),
        jax.ShapeDtypeStruct((D, 3 * D), bf16),
        jax.ShapeDtypeStruct((DH, DH, H), bf16),
        jax.ShapeDtypeStruct((D, D), bf16),
        jax.ShapeDtypeStruct((D, F), bf16),
        jax.ShapeDtypeStruct((D, F), bf16),
        jax.ShapeDtypeStruct((F, D), bf16),
    )
    any_spec = pl.BlockSpec(memory_space=pl.ANY)
    outs = pl.pallas_call(
        _kernel,
        out_shape=out_shape,
        in_specs=[any_spec] * 8,
        out_specs=tuple([any_spec] * 8),
        scratch_shapes=scratch,
        compiler_params=pltpu.CompilerParams(vmem_limit_bytes=120 * 1024 * 1024),
    )(A_x, A_wqkv, jnp.transpose(A_w_phi, (1, 2, 0)), A_wo, B_w_gate, B_w_up, B_w_down, grad_out)
    out, gx, dwqkv, dwphi_t, dwo, dwg, dwu, dwd = outs
    return (out, gx, dwqkv, jnp.transpose(dwphi_t, (2, 0, 1)), dwo, dwg, dwu, dwd)
```
